```python
import jax
import jax.numpy as jnp

def _softmax(x, axis=-1):
    return jax.nn.softmax(x, axis=axis)
def _gelu(x):
    return jax.nn.gelu(x, approximate=True)
def _silu(x):
    return jax.nn.silu(x)
def _sigmoid(x):
    return jax.nn.sigmoid(x)
def _layernorm(x, axis=-1, eps=1e-5):
    m = jnp.mean(x, axis=axis, keepdims=True)
    v = jnp.var(x, axis=axis, keepdims=True)
    return (x - m) / jnp.sqrt(v + eps)
def _scatter_add(tgt, idx, src, axis=0):
    return tgt.at[idx].add(src)
def _segment_sum(src, seg, n):
    return jax.ops.segment_sum(src, seg, n)
class _Rng:
    def __init__(self, key):
        self._k = key
    def _next(self):
        self._k, sub = jax.random.split(self._k)
        return sub
    def normal(self, shape):
        return jax.random.normal(self._next(), shape, dtype=jnp.bfloat16)
    def randint(self, lo, hi, shape):
        return jax.random.randint(self._next(), shape, lo, hi, dtype=jnp.int32)
    def uniform(self, shape, lo=0.0, hi=1.0):
        return jax.random.uniform(self._next(), shape, jnp.bfloat16, lo, hi)
    def permutation(self, n):
        return jax.random.permutation(self._next(), n)


kernel_name = 'recurrent_scan__sliding_local_dilated__glu_gated_swiglu__prompt'

def setup_inputs():
    _rng = _Rng(jax.random.key(int.from_bytes(__import__("os").urandom(4), "little")))
    _w = (lambda a: (lambda t: t.astype(jnp.bfloat16) if jnp.issubdtype(t.dtype, jnp.floating) else t)(jnp.asarray(a)))
    def _A_setup():
        B, S, D = 1, 2048, 1024
        return {
            "x": _w((lambda *s: _rng.normal(s) * 0.05)(B, S, D)),
            "wqkv": _w((lambda *s: _rng.normal(s) * 0.05)(D, 3 * D)),
            "wo": _w((lambda *s: _rng.normal(s) * 0.05)(D, D)),
        }
    _A_in = _A_setup()

    def _B_setup():
        B, S, D, F = 1, 2048, 1024, 3584
        return {
            "x": _w((lambda *s: _rng.normal(s) * 0.05)(B, S, D)),
            "w1": _w((lambda *s: _rng.normal(s) * 0.05)(D, F) * (2.0 / D) ** 0.5),
            "w3": _w((lambda *s: _rng.normal(s) * 0.05)(D, F) * (2.0 / D) ** 0.5),
            "w2": _w((lambda *s: _rng.normal(s) * 0.05)(F, D) * (2.0 / F) ** 0.5),
        }
    _B_in = _B_setup()

    return {
        "A_x": _A_in["x"],
        "A_wqkv": _A_in["wqkv"],
        "A_wo": _A_in["wo"],
        "B_x": _B_in["x"],
        "B_w1": _B_in["w1"],
        "B_w3": _B_in["w3"],
        "B_w2": _B_in["w2"],
    }

def reference(A_x, A_wqkv, A_wo, B_x, B_w1, B_w3, B_w2):
    def _A_ref(x, wqkv, wo):
        B, S, D = x.shape
        H = 32; Dh = D // H
        W, dil = 8, 2
        qkv = (lambda x, *d: x.transpose(*d))((x @ wqkv).reshape(B, S, 3, H, Dh), 2, 0, 3, 1, 4)
        q, k, v = qkv[0], qkv[1], qkv[2]
        scale = Dh ** -0.5
        pos = jnp.arange(S)
        off = jnp.arange(W) * dil
        idx = pos[:, None] - off[None, :]
        mask = idx >= 0
        idx_c = jnp.where(mask, idx, 0).reshape(-1)
        kg = k[:, :, idx_c, :].reshape(B, H, S, W, Dh)
        vg = v[:, :, idx_c, :].reshape(B, H, S, W, Dh)
        logits = jnp.einsum("bhsd,bhswd->bhsw", q, kg) * scale
        logits = jnp.where(mask[None, None, :, :], logits, -1e9)
        attn = _softmax(logits, axis=-1)
        o = jnp.einsum("bhsw,bhswd->bhsd", attn, vg)
        return (lambda x, *d: x.transpose(*d))(o, 0, 2, 1, 3).reshape(B, S, D) @ wo

    def _B_ref(x, w1, w3, w2):
        gate = jnp.einsum("bsd,df->bsf", x, w1)
        up = jnp.einsum("bsd,df->bsf", x, w3)
        h = _silu(gate) * up
        out = jnp.einsum("bsf,fd->bsd", h, w2)
        return out

    x = A_x
    xn = _layernorm(x, axis=-1)
    s = _A_ref(xn, A_wqkv, A_wo)
    g = _silu(_B_ref(xn, B_w1, B_w3, B_w2))
    return x + s * g
```

```python
import contextlib
import functools

import jax
import jax.numpy as jnp
import numpy as np
from jax import lax
import jax.experimental.pallas as pl
import jax.experimental.pallas.tpu as pltpu

S, D, F = 2048, 1024, 3584
H, DH, WIN, DIL = 32, 32, 8, 2
HS = S // 2
HD = D // 2
HF = F // 2
NCH = HF // 128
F32, BF16 = jnp.float32, jnp.bfloat16
EPS = 1e-5
SCALE = DH ** -0.5
PAD = 16


def _dot(a, b):
    return jnp.dot(a, b, preferred_element_type=F32)


def _lhs_combos(a11, a12, a21, a22):
    return [a11 + a22, a21 + a22, a11, a22, a11 + a12, a21 - a11, a12 - a22]


def _rhs_combos(b11, b12, b21, b22):
    return [b11 + b22, b11, b12 - b22, b21 - b11, b22, b11 + b12, b21 + b22]


def _out_combos(m):
    m1, m2, m3, m4, m5, m6, m7 = m
    c11 = (m1 + m4) + (m7 - m5)
    c12 = m3 + m5
    c21 = m2 + m4
    c22 = (m1 + m3) + (m6 - m2)
    return c11, c12, c21, c22


def _after(tok, r, never):
    if tok is None:
        return r
    head = jnp.where(never, tok.astype(r.dtype), r[0:16])
    return jnp.concatenate([head, r[16:]], axis=0)


def _pk(x):
    return pltpu.bitcast(x.astype(BF16), jnp.uint32)


def _unpk(x):
    return pltpu.bitcast(x, BF16)


def _silu(x):
    hx = 0.5 * x
    return hx + hx * jnp.tanh(hx)


def make_kernel(NC0, RP, AT_ROWS, AT_G, QN, SPREAD=None, scopes=False):
    NRP = HS // RP
    NMAIN = NCH - NC0
    assert NMAIN * AT_ROWS >= HS

    def scope(name):
        return jax.named_scope(name) if scopes else contextlib.nullcontext()

    def kernel(x_hbm, wqkv_hbm, wo_hbm, w1_hbm, w3_hbm, w2_hbm, out_hbm,
               x_v, xl, wqkv_r, w13_0, w13_r, w2_r, wo_r, wo_t, hl, ol, qkv, rq, sems, osem):
        def x_copy(i, half):
            r = half * HS + i * RP
            return pltpu.make_async_copy(x_hbm.at[pl.ds(r, RP)], x_v.at[pl.ds(r, RP)], sems.at[half * NRP + i])

        SB = 2 * NRP

        def wqkv_copy(p):
            return pltpu.make_async_copy(wqkv_hbm.at[:, pl.ds(p * D, D)], wqkv_r.at[p], sems.at[SB + p])

        def w13_copies(j, dst, sem0):
            c = pl.multiple_of(j * 128, 128)
            return [
                pltpu.make_async_copy(w1_hbm.at[:, pl.ds(c, 128)], dst.at[0], sems.at[sem0]),
                pltpu.make_async_copy(w3_hbm.at[:, pl.ds(c, 128)], dst.at[1], sems.at[sem0 + 1]),
                pltpu.make_async_copy(w1_hbm.at[:, pl.ds(HF + c, 128)], dst.at[2], sems.at[sem0 + 2]),
                pltpu.make_async_copy(w3_hbm.at[:, pl.ds(HF + c, 128)], dst.at[3], sems.at[sem0 + 3]),
            ]

        SEM_W0 = SB + 3
        SEM_W = SEM_W0 + 4 * NC0
        SEM_W2 = SEM_W + 8
        SEM_WO = SEM_W2 + 8

        def w2_copy(n):
            return pltpu.make_async_copy(w2_hbm.at[:, pl.ds(n * 128, 128)], w2_r.at[n], sems.at[SEM_W2 + n])

        def wo_copy(n):
            return pltpu.make_async_copy(wo_hbm.at[:, pl.ds(n * 128, 128)], wo_r.at[n], sems.at[SEM_WO + n])

        x_copy(0, 0).start()
        x_copy(0, 1).start()
        for c0 in range(NC0):
            for cp in w13_copies(c0, w13_0.at[c0], SEM_W0 + 4 * c0):
                cp.start()
        for i in range(1, NRP):
            x_copy(i, 0).start()
            x_copy(i, 1).start()
        for p in range(3):
            wqkv_copy(p).start()
        for cp in w13_copies(NC0, w13_r.at[0], SEM_W):
            cp.start()
        for n in range(8):
            w2_copy(n).start()
        for n in range(8):
            wo_copy(n).start()

        for j in range(8, 24):
            qkv[j, 0:PAD, :] = jnp.zeros((PAD, 128), F32)

        def ln_rows(r):
            xv = x_v[pl.ds(r, RP), :].astype(F32)
            mean = jnp.sum(xv, axis=-1, keepdims=True) * (1.0 / D)
            xc = xv - mean
            var = jnp.sum(xc * xc, axis=-1, keepdims=True) * (1.0 / D)
            return xc * lax.rsqrt(var + EPS)

        def ln_pair(r):
            top = ln_rows(r)
            bot = ln_rows(HS + r)
            ops = _lhs_combos(top[:, :HD], top[:, HD:], bot[:, :HD], bot[:, HD:])
            for t in range(7):
                xl[t, pl.ds(r // 2, RP // 2), :] = _pk(ops[t])

        def never_mask(i):
            return lax.broadcasted_iota(jnp.int32, (16, 128), 1) < (i - 1048576)

        def gate_up(lhs, w, fillers=None, never=None):
            hs = []
            ends = {}
            for half in range(2):
                w1, w3 = w.at[2 * half], w.at[2 * half + 1]
                rhs = _rhs_combos(w1[0:HD, :].astype(F32), w3[0:HD, :].astype(F32),
                                  w1[HD:D, :].astype(F32), w3[HD:D, :].astype(F32))
                m = []
                for t in range(7):
                    u = half * 7 + t
                    r = rhs[t].astype(BF16)
                    for tok in ends.pop(u, []):
                        r = _after(tok, r, never)
                    m.append(_dot(lhs(t), r))
                    for fn, use_start, row, end in (fillers or {}).get(u, []):
                        tok = fn(m[-1][row:row + 16] if use_start else None)
                        if end is not None:
                            ends.setdefault(end, []).append(tok)
                g_top, u_top, g_bot, u_bot = _out_combos(m)
                hs.append((_silu(g_top) * u_top, _silu(g_bot) * u_bot))
            return _lhs_combos(hs[0][0], hs[1][0], hs[0][1], hs[1][1])

        with scope("P_ln0"):
            x_copy(0, 0).wait()
            x_copy(0, 1).wait()
            ln_pair(0)
            for c0 in range(NC0):
                for cp in w13_copies(c0, w13_0.at[c0], SEM_W0 + 4 * c0):
                    cp.wait()

        def first_body(i, carry):
            for ii in range(1, NRP):
                @pl.when(i + 1 == ii)
                def _():
                    x_copy(ii, 0).wait()
                    x_copy(ii, 1).wait()
            r = pl.multiple_of(i * RP, RP)
            rn = pl.multiple_of(jnp.minimum(i + 1, NRP - 1) * RP, RP)
            rh = pl.multiple_of(i * (RP // 2), RP // 2)
            rnh = pl.multiple_of(jnp.minimum(i + 1, NRP - 1) * (RP // 2), RP // 2)
            lhs_vals = [_unpk(xl[t, pl.ds(rh, RP // 2), :]) for t in range(7)]
            top = ln_rows(rn)
            bot = ln_rows(HS + rn)
            nxt = _lhs_combos(top[:, :HD], top[:, HD:], bot[:, :HD], bot[:, HD:])
            for c0 in range(NC0):
                ops = gate_up(lambda t: lhs_vals[t], w13_0.at[c0])
                for t in range(7):
                    hl[c0, t, pl.ds(rh, RP // 2), :] = _pk(ops[t])
            for t in range(7):
                xl[t, pl.ds(rnh, RP // 2), :] = _pk(nxt[t])
            return carry

        with scope("P_first"):
            lax.fori_loop(0, NRP, first_body, 0)

        NQ = 4 // QN

        def qkv_prep(it):
            p = it // NQ
            i0 = (it % NQ) * QN
            ln = lax.broadcasted_iota(jnp.int32, (D // 2, 128), 1)
            pos = (ln >> 2) & 7
            ys = []
            for j in range(8):
                v = pltpu.bitcast(wqkv_r[p, :, j * 128:(j + 1) * 128], jnp.uint32)
                ys.append(v if j == 0 else pltpu.roll(v, 4 * j, 1))
            hh_full = (ln >> 1) & 31
            base = ((hh_full & 3) * 8 + (hh_full >> 2))
            low = (ln >> 6) * 2 + (ln & 1)

            def column_tile(i):
                sel = (pos - i) & 7
                z = ys[0]
                for j in range(1, 8):
                    z = jnp.where(sel == j, ys[j], z)
                src = (((base + i) & 31) << 2) + low
                return pltpu.bitcast(jnp.take_along_axis(z, src, axis=1), BF16).astype(F32)

            out = []
            for di in range(QN):
                left = column_tile(i0 + di)
                right = column_tile(i0 + di + 4)
                rhs = _rhs_combos(left[:HD], right[:HD], left[HD:], right[HD:])
                out.append([_pk(r) for r in rhs])
            return out

        def qkv_store_prep(vals):
            for di in range(QN):
                for t in range(7):
                    rq[di, t] = vals[di][t]

        def qkv_body(it, carry):
            for pp in range(1, 3):
                @pl.when(it + 1 == pp * NQ)
                def _():
                    wqkv_copy(pp).wait()
            p = it // NQ
            i0 = (it % NQ) * QN
            cur = [[_unpk(rq[di, t]) for t in range(7)] for di in range(QN)]
            nxt = qkv_prep(jnp.minimum(it + 1, 3 * NQ - 1))
            for di in range(QN):
                i = i0 + di
                m = [_dot(_unpk(xl[t]), cur[di][t]) for t in range(7)]
                c11, c12, c21, c22 = _out_combos(m)
                qkv[p * 8 + i, PAD:PAD + HS, :] = c11
                qkv[p * 8 + 4 + i, PAD:PAD + HS, :] = c12
                qkv[p * 8 + i, PAD + HS:PAD + S, :] = c21
                qkv[p * 8 + 4 + i, PAD + HS:PAD + S, :] = c22
            qkv_store_prep(nxt)
            return carry

        with scope("P_qkv0"):
            wqkv_copy(0).wait()
            qkv_store_prep(qkv_prep(0))
        with scope("P_qkv"):
            lax.fori_loop(0, 3 * NQ, qkv_body, 0)

        def attn_rows(r, n, tok, never):
            ln = lax.broadcasted_iota(jnp.int32, (n, 128), 1)
            row = lax.broadcasted_iota(jnp.int32, (n, 128), 0) + r
            q = [qkv[j, pl.ds(r + PAD, n), :] for j in range(8)]
            if tok is not None:
                tk = jnp.concatenate([tok] * (n // 16), axis=0) if n > 16 else tok[0:n]
                nv = jnp.concatenate([never] * (n // 16), axis=0) if n > 16 else never[0:n]
                q = [jnp.where(nv, tk, qq) for qq in q]
            logits = []
            for w in range(WIN):
                p = None
                for j in range(8):
                    t = q[j] * qkv[8 + j, pl.ds(r + (PAD - DIL * w), n), :]
                    p = t if p is None else p + t
                p = p + pltpu.roll(p, 64, 1)
                p = p + jnp.take_along_axis(p, ln ^ 1, axis=1)
                p = p * SCALE
                if w > 0:
                    p = jnp.where(row >= DIL * w, p, -1e9)
                logits.append(p)
            mx = logits[0]
            for w in range(1, WIN):
                mx = jnp.maximum(mx, logits[w])
            es = [jnp.exp(l - mx) for l in logits]
            den = es[0]
            for w in range(1, WIN):
                den = den + es[w]
            inv = 1.0 / den
            outs = []
            for j in range(8):
                o = None
                for w in range(WIN):
                    t = es[w] * qkv[16 + j, pl.ds(r + (PAD - DIL * w), n), :]
                    o = t if o is None else o + t
                outs.append(o * inv)
            return outs

        def attn_group(r, rh, n, tok=None, never=None):
            top = attn_rows(r, n, tok, never)
            bot = attn_rows(HS + r, n, tok, never)
            tok = None
            for j in range(4):
                ops = _lhs_combos(top[j], top[4 + j], bot[j], bot[4 + j])
                for t in range(7):
                    ol[t, pl.ds(rh, n // 2), j * 128:(j + 1) * 128] = _pk(ops[t])
                part = ops[0] + ops[4] + ops[1]
                tok = part if tok is None else tok + part
            return tok[n - 16:n] if n >= 16 else jnp.concatenate([tok, tok], axis=0)

        def main_body(jj, carry):
            j = jj + NC0
            slot = jj & 1
            for cp in w13_copies(j, w13_r.at[slot], SEM_W + 4 * slot):
                cp.wait()

            @pl.when(jj + 1 < NMAIN)
            def _():
                for cp in w13_copies(j + 1, w13_r.at[1 - slot], SEM_W + 4 * (1 - slot)):
                    cp.start()

            a0h = pl.multiple_of(jnp.minimum(jj * (AT_ROWS // 2), (HS - AT_ROWS) // 2), 8)
            a0 = pl.multiple_of(a0h * 2, 16)
            ng = AT_ROWS // AT_G
            if SPREAD:
                fillers = {}
                never = never_mask(jj)
                assert len(SPREAD) == ng
                for g, (place, use_start, row, end) in enumerate(SPREAD):
                    def fn(tok, g=g):
                        return attn_group(a0 + g * AT_G, a0h + g * (AT_G // 2), AT_G, tok, never)
                    fillers.setdefault(place, []).append((fn, use_start, row, end))
                ops = gate_up(lambda t: _unpk(xl[t]), w13_r.at[slot], fillers, never)
            else:
                ops = gate_up(lambda t: _unpk(xl[t]), w13_r.at[slot])
                for g in range(ng):
                    attn_group(a0 + g * AT_G, a0h + g * (AT_G // 2), AT_G)
            for t in range(7):
                hl[j, t] = _pk(ops[t])
            return carry

        with scope("P_main"):
            lax.fori_loop(0, NMAIN, main_body, 0)

        def out_copy(n, half):
            c = pl.multiple_of((half * 4 + n) * 128, 128)
            return pltpu.make_async_copy(x_v.at[:, pl.ds(c, 128)], out_hbm.at[:, pl.ds(c, 128)], osem.at[half * 4 + n])

        for n in range(8):
            w2_copy(n).wait()
            wo_copy(n).wait()

        def fin_body(n, carry):
            wo_t[0] = pltpu.bitcast(wo_r[n], jnp.uint32)
            wo_t[1] = pltpu.bitcast(wo_r[4 + n], jnp.uint32)

            def rows(side, lo):
                parts = [wo_t[side, pl.ds(dd, 32, stride=16), :] for dd in range(lo, lo + 8)]
                return pltpu.bitcast(jnp.concatenate(parts, axis=0), BF16).astype(F32)
            rhs = _rhs_combos(rows(0, 0), rows(1, 0), rows(0, 8), rows(1, 8))
            m = [_dot(_unpk(ol[t]), rhs[t].astype(BF16)) for t in range(7)]
            s_q = _out_combos(m)

            rhs = _rhs_combos(w2_r[n, 0:HF, :].astype(F32), w2_r[4 + n, 0:HF, :].astype(F32),
                              w2_r[n, HF:F, :].astype(F32), w2_r[4 + n, HF:F, :].astype(F32))
            m = []
            for t in range(7):
                lhs = jnp.concatenate([_unpk(hl[j, t]) for j in range(NCH)], axis=1)
                m.append(_dot(lhs, rhs[t].astype(BF16)))
            b_q = _out_combos(m)
            ca = pl.multiple_of(n * 128, 128)
            cb = pl.multiple_of((4 + n) * 128, 128)
            for (r0, c0), sv, bv in zip(((0, ca), (0, cb), (HS, ca), (HS, cb)), s_q, b_q):
                idx = (pl.ds(r0, HS), pl.ds(c0, 128))
                x_v[idx] = (x_v[idx].astype(F32) + sv * _silu(bv)).astype(BF16)
            out_copy(n, 0).start()
            out_copy(n, 1).start()
            return carry

        with scope("P_fin"):
            lax.fori_loop(0, 4, fin_body, 0)
            for n in range(4):
                out_copy(n, 0).wait()
                out_copy(n, 1).wait()

    NRP = HS // RP
    scratch = [
        pltpu.VMEM((S, D), BF16),
        pltpu.VMEM((7, HS // 2, HD), jnp.uint32),
        pltpu.VMEM((3, D, D), BF16),
        pltpu.VMEM((NC0, 4, D, 128), BF16),
        pltpu.VMEM((2, 4, D, 128), BF16),
        pltpu.VMEM((8, F, 128), BF16),
        pltpu.VMEM((8, D, 128), BF16),
        pltpu.VMEM((2, D // 2, 128), jnp.uint32),
        pltpu.VMEM((NCH, 7, HS // 2, 128), jnp.uint32),
        pltpu.VMEM((7, HS // 2, HD), jnp.uint32),
        pltpu.VMEM((24, S + PAD, 128), F32),
        pltpu.VMEM((QN, 7, HD // 2, 128), jnp.uint32),
        pltpu.SemaphoreType.DMA((2 * NRP + 3 + 4 * NC0 + 24,)),
        pltpu.SemaphoreType.DMA((8,)),
    ]
    return kernel, scratch


_CFG = dict(NC0=2, RP=256, QN=1, AT_ROWS=96, AT_G=16)


@jax.jit
def pallas_recurrent_scan__sliding_local_dilated__glu_gated_swiglu__prompt_kernel(
    A_x: jax.Array,
    A_wqkv: jax.Array,
    A_wo: jax.Array,
    B_x: jax.Array,
    B_w1: jax.Array,
    B_w3: jax.Array,
    B_w2: jax.Array,
):
    del B_x
    kernel, scratch = make_kernel(**_CFG)
    any_spec = pl.BlockSpec(memory_space=pl.ANY)
    out = pl.pallas_call(
        kernel,
        out_shape=jax.ShapeDtypeStruct((S, D), BF16),
        in_specs=[any_spec] * 6,
        out_specs=any_spec,
        scratch_shapes=scratch,
        compiler_params=pltpu.CompilerParams(
            vmem_limit_bytes=120 * 2**20,
            flags={"XLA_TPU_EVENLY_DISTRIBUTE_CRITICAL_NODES": True},
        ),
    )(A_x.reshape(S, D), A_wqkv, A_wo, B_w1, B_w3, B_w2)
    return out.reshape(1, S, D)
```

```python
import contextlib

import jax
import jax.numpy as jnp
from jax import lax
import jax.experimental.pallas as pl
import jax.experimental.pallas.tpu as pltpu

S, D, F = 2048, 1024, 3584
H, DH, WIN, DIL = 32, 32, 8, 2
HS = S // 2
HD = D // 2
QD = D // 4
HF = F // 2
NCH = HF // 128
F32, BF16 = jnp.float32, jnp.bfloat16
EPS = 1e-5
SCALE = DH ** -0.5
LOG2E = 1.4426950408889634
MASKED = -1e9 * LOG2E
PAD = 16


def _dot(a, b):
    return jnp.dot(a, b, preferred_element_type=F32)


def _lhs_combos(a11, a12, a21, a22):
    return [a11 + a22, a21 + a22, a11, a22, a11 + a12, a21 - a11, a12 - a22]


def _rhs_combos(b11, b12, b21, b22):
    return [_unpk(v) for v in _rhs_words(*[_words(b) for b in (b11, b12, b21, b22)])]


def _lin_combos(b11, b12, b21, b22):
    return [b11 + b22, b11, b12 - b22, b21 - b11, b22, b11 + b12, b21 + b22]


def _eo(w):
    return (pltpu.bitcast(w << 16, F32), pltpu.bitcast(w & jnp.uint32(0xFFFF0000), F32))


def _pk_eo(e, o):
    return pltpu.pack_elementwise([e, o], packed_dtype=BF16)


def _words(x):
    return pltpu.bitcast(x, jnp.uint32)


def _rhs_words(b11, b12, b21, b22):
    eo = [_eo(b) for b in (b11, b12, b21, b22)]
    ce = _lin_combos(*[v[0] for v in eo])
    co = _lin_combos(*[v[1] for v in eo])
    return [b11 if t == 1 else b22 if t == 4 else _pk_eo(ce[t], co[t]) for t in range(7)]


def _lhs_words(a11, a12, a21, a22):
    ce = _lhs_combos(a11[0], a12[0], a21[0], a22[0])
    co = _lhs_combos(a11[1], a12[1], a21[1], a22[1])
    return [_pk_eo(e, o) for e, o in zip(ce, co)]


def _products(lhs, rhs, order):
    m = [None] * 7
    for t in order:
        m[t] = _dot(lhs(t), rhs[t])
    return m


def _out_combos(m):
    m1, m2, m3, m4, m5, m6, m7 = m
    c11 = (m1 + m4) + (m7 - m5)
    c12 = m3 + m5
    c21 = m2 + m4
    c22 = (m1 + m3) + (m6 - m2)
    return c11, c12, c21, c22


def _pk(x):
    return pltpu.bitcast(x.astype(BF16), jnp.uint32)


def _unpk(x):
    return pltpu.bitcast(x, BF16)


def _silu(x):
    hx = 0.5 * x
    return hx + hx * jnp.tanh(hx)


def make_kernel(RQ=128, LG=32, PREP=1, RTRIP=0, IORDER=(4, 1, 2, 3, 0, 5, 6), AT_G=16, ORDER=(1, 4, 0, 2, 3, 5, 6), QPOS=2, ATPOS=0, CHAIN=4, MIDWAIT=0, DORDER=None, FORDER=None, QORDER=None, WOT=0, GATE=8, LOG2=1, scopes=False):
    DORDER = DORDER or ORDER
    FORDER = FORDER or ORDER
    QORDER = QORDER or ORDER
    NC0 = 2
    QS = S // 4
    NRP = QS // RQ
    NMAIN = NCH - NC0
    AT_ROWS = HS // 4

    def scope(name):
        return jax.named_scope(name) if scopes else contextlib.nullcontext()

    def kernel(x_hbm, wqkv_hbm, wo_hbm, w1_hbm, w3_hbm, w2_hbm, out_hbm,
               x_v, w2_r, wo_r, hl, qkv, sems, osem):
        SB = 4 * NRP
        SEM_W0 = SB + 3
        SEM_W = SEM_W0 + 4 * NC0
        SEM_W2 = SEM_W + 8
        SEM_WO = SEM_W2 + 8

        def w2_copy(n):
            return pltpu.make_async_copy(w2_hbm.at[:, pl.ds(n * 128, 128)], w2_r.at[n], sems.at[SEM_W2 + n])

        def wo_copy(n):
            return pltpu.make_async_copy(wo_hbm.at[:, pl.ds(n * 128, 128)], wo_r.at[n], sems.at[SEM_WO + n])

        def phase_a(xl, xl2, rg, hs_v, wqkv_r, w13_0, w13_r):
            def x_copy(i, q):
                r = q * QS + i * RQ
                return pltpu.make_async_copy(x_hbm.at[pl.ds(r, RQ)], x_v.at[pl.ds(r, RQ)], sems.at[q * NRP + i])

            def wqkv_copy(p):
                return pltpu.make_async_copy(wqkv_hbm.at[:, pl.ds(p * D, D)], wqkv_r.at[p], sems.at[SB + p])

            def w13_copies(j, dst, sem0):
                c = pl.multiple_of(j * 128, 128)
                return [
                    pltpu.make_async_copy(w1_hbm.at[:, pl.ds(c, 128)], dst.at[0], sems.at[sem0]),
                    pltpu.make_async_copy(w3_hbm.at[:, pl.ds(c, 128)], dst.at[2], sems.at[sem0 + 1]),
                    pltpu.make_async_copy(w1_hbm.at[:, pl.ds(HF + c, 128)], dst.at[1], sems.at[sem0 + 2]),
                    pltpu.make_async_copy(w3_hbm.at[:, pl.ds(HF + c, 128)], dst.at[3], sems.at[sem0 + 3]),
                ]

            def ln_rows(r, n):
                outs = []
                for xv in _eo(_words(x_v[pl.ds(r, n), :])):
                    mean = jnp.sum(xv, axis=-1, keepdims=True) * (1.0 / D)
                    xc = xv - mean
                    var = jnp.sum(xc * xc, axis=-1, keepdims=True) * (1.0 / D)
                    outs.append(xc * lax.rsqrt(var + EPS))
                return outs

            def ln_vals(r, two=True):
                p1a, p1b = [[] for _ in range(7)], [[] for _ in range(7)]
                p2 = [[] for _ in range(49)]
                for g in range(0, RQ, LG):
                    rows = [ln_rows(q * QS + r + g, LG) for q in range(4)]
                    la, lb, inner = [], [], []
                    for e in range(2):
                        rw = [v[e] for v in rows]
                        la.append(_lhs_combos(rw[0][:, :HD], rw[0][:, HD:], rw[2][:, :HD], rw[2][:, HD:]))
                        lb.append(_lhs_combos(rw[1][:, :HD], rw[1][:, HD:], rw[3][:, :HD], rw[3][:, HD:]))
                    for t in range(7):
                        p1a[t].append(_pk_eo(la[0][t], la[1][t]))
                        p1b[t].append(_pk_eo(lb[0][t], lb[1][t]))
                        if two:
                            inner = [_lhs_combos(la[e][t][:, :QD], la[e][t][:, QD:], lb[e][t][:, :QD], lb[e][t][:, QD:])
                                     for e in range(2)]
                            for u in range(7):
                                p2[t * 7 + u].append(_pk_eo(inner[0][u], inner[1][u]))
                cat = lambda ps: [jnp.concatenate(p, axis=0) if len(p) > 1 else p[0] for p in ps]
                return cat(p1a), cat(p1b), cat(p2) if two else []

            def split_rows(slot, v):
                n = v.shape[0]
                hs_v[slot, 0:n, :] = v
                return [hs_v[slot, pl.ds(e, n // 2, stride=2), :] for e in range(2)]

            def ln_store(rh, vals):
                va, vb, v2 = vals
                for t in range(7):
                    xl[t, pl.ds(rh, RQ // 2), :] = va[t]
                    xl[t, pl.ds(QS // 2 + rh, RQ // 2), :] = vb[t]
                for t in range(len(v2)):
                    xl2[t, pl.ds(rh, RQ // 2), :] = v2[t]

            def first_rhs(w, half):
                w1, w3 = w.at[half], w.at[2 + half]
                return _rhs_words(*[_words(v) for v in (w1[0:HD, :], w3[0:HD, :], w1[HD:D, :], w3[HD:D, :])])

            def gate_up(lhs, c0):
                hs = []
                for half in range(2):
                    if PREP:
                        rhs = [_unpk(rg[c0, half, t]) for t in range(7)]
                    else:
                        rhs = [_unpk(v) for v in first_rhs(w13_0.at[c0], half)]
                    g_top, u_top, g_bot, u_bot = _out_combos(_products(lhs, rhs, ORDER))
                    if RTRIP:
                        hs.append((split_rows(4 * c0 + 2 * half, _silu(g_top) * u_top),
                                   split_rows(4 * c0 + 2 * half + 1, _silu(g_bot) * u_bot)))
                    else:
                        hs.append((_silu(g_top) * u_top, _silu(g_bot) * u_bot))
                if RTRIP:
                    return _lhs_words(hs[0][0], hs[1][0], hs[0][1], hs[1][1])
                return [_pk(v) for v in _lhs_combos(hs[0][0], hs[1][0], hs[0][1], hs[1][1])]

            def gate_up2(w):
                blk = lambda kq, nq: _eo(_words(w[nq, kq * QD:(kq + 1) * QD, :]))
                big = [[[[blk(2 * kh + a, 2 * nh + b) for b in range(2)] for a in range(2)] for nh in range(2)] for kh in range(2)]
                mm = [None] * 7
                for t in ORDER:
                    inner = []
                    for e in range(2):
                        r = [[_lin_combos(big[0][0][a][b][e], big[0][1][a][b][e], big[1][0][a][b][e], big[1][1][a][b][e])[t]
                              for b in range(2)] for a in range(2)]
                        inner.append(_lin_combos(r[0][0], r[0][1], r[1][0], r[1][1]))
                    rr = [_unpk(_pk_eo(ve, vo)) for ve, vo in zip(*inner)]
                    c = _out_combos(_products(lambda u: _unpk(xl2[t * 7 + u]), rr, IORDER))
                    mm[t] = [[c[0], c[1]], [c[2], c[3]]]
                cc = [[None] * 4 for _ in range(4)]
                for a in range(2):
                    for b in range(2):
                        o11, o12, o21, o22 = _out_combos([mm[t][a][b] for t in range(7)])
                        cc[a][b], cc[a][2 + b], cc[2 + a][b], cc[2 + a][2 + b] = o11, o12, o21, o22
                if not RTRIP:
                    h = [[_silu(cc[q][b]) * cc[q][2 + b] for b in range(2)] for q in range(4)]
                    return [[_pk(v) for v in _lhs_combos(h[a][0], h[a][1], h[2 + a][0], h[2 + a][1])] for a in range(2)]
                h = [[split_rows(2 * q + b, _silu(cc[q][b]) * cc[q][2 + b]) for b in range(2)] for q in range(4)]
                return [_lhs_words(h[a][0], h[a][1], h[2 + a][0], h[2 + a][1]) for a in range(2)]

            with scope("P_ln0"):
                for q in range(4):
                    x_copy(0, q).start()
                for c0 in range(NC0):
                    for cp in w13_copies(c0, w13_0.at[c0], SEM_W0 + 4 * c0):
                        cp.start()
                for j in range(8, 24):
                    qkv[j, 0:PAD, :] = jnp.zeros((PAD, 128), F32)
                for q in range(4):
                    x_copy(0, q).wait()
                for i in range(1, NRP):
                    for q in range(4):
                        x_copy(i, q).start()
                ln_store(0, ln_vals(0, False))
                for c0 in range(NC0):
                    for cp in w13_copies(c0, w13_0.at[c0], SEM_W0 + 4 * c0):
                        cp.wait()
                    if PREP:
                        for half in range(2):
                            rhs = first_rhs(w13_0.at[c0], half)
                            for t in range(7):
                                rg[c0, half, t] = rhs[t]
                for cp in w13_copies(NC0, w13_r.at[0], SEM_W):
                    cp.start()
                for p in range(3):
                    wqkv_copy(p).start()
                for n in range(8):
                    w2_copy(n).start()
                for n in range(8):
                    wo_copy(n).start()

            def first_body(i, carry):
                for ii in range(1, NRP):
                    @pl.when(i + 1 == ii)
                    def _():
                        for q in range(4):
                            x_copy(ii, q).wait()
                inext = jnp.where(i + 1 == NRP, 0, i + 1)
                rn = pl.multiple_of(inext * RQ, RQ)
                rh = pl.multiple_of(i * (RQ // 2), RQ // 2)
                rnh = pl.multiple_of(inext * (RQ // 2), RQ // 2)
                lhs_vals = [_unpk(jnp.concatenate([xl[t, pl.ds(rh, RQ // 2), :], xl[t, pl.ds(QS // 2 + rh, RQ // 2), :]], axis=0))
                            for t in range(7)]
                nxt = ln_vals(rn)
                for c0 in range(NC0):
                    ops = gate_up(lambda t: lhs_vals[t], c0)
                    for t in range(7):
                        pk = ops[t]
                        hl[c0, t, pl.ds(rh, RQ // 2), :] = pk[0:RQ // 2]
                        hl[c0, t, pl.ds(QS // 2 + rh, RQ // 2), :] = pk[RQ // 2:RQ]
                ln_store(rnh, nxt)
                return carry

            with scope("P_first"):
                lax.fori_loop(0, NRP, first_body, 0)

            def qkv_tile(p, i):
                ln = lax.broadcasted_iota(jnp.int32, (D // 2, 128), 1)
                pos = (ln >> 2) & 7
                ys = []
                for j in range(8):
                    v = pltpu.bitcast(wqkv_r[p, :, j * 128:(j + 1) * 128], jnp.uint32)
                    ys.append(v if j == 0 else pltpu.roll(v, 4 * j, 1))
                hh_full = (ln >> 1) & 31
                base = ((hh_full & 3) * 8 + (hh_full >> 2))
                low = (ln >> 6) * 2 + (ln & 1)

                def column_tile(ii):
                    sel = (pos - ii) & 7
                    z = ys[0]
                    for j in range(1, 8):
                        z = jnp.where(sel == j, ys[j], z)
                    src = (((base + ii) & 31) << 2) + low
                    return jnp.take_along_axis(z, src, axis=1)

                left = column_tile(i)
                right = column_tile(i + 4)
                rhs = [_unpk(v) for v in _rhs_words(left[:QD], right[:QD], left[QD:], right[QD:])]
                c11, c12, c21, c22 = _out_combos(_products(lambda t: _unpk(xl[t]), rhs, QORDER))
                if LOG2:
                    sc = jnp.where(p == 0, SCALE * LOG2E, 1.0).astype(F32)
                    c11, c12, c21, c22 = c11 * sc, c12 * sc, c21 * sc, c22 * sc
                qkv[p * 8 + i, PAD:PAD + HS, :] = c11
                qkv[p * 8 + 4 + i, PAD:PAD + HS, :] = c12
                qkv[p * 8 + i, PAD + HS:PAD + S, :] = c21
                qkv[p * 8 + 4 + i, PAD + HS:PAD + S, :] = c22

            def main_body(jj, carry):
                j = jj + NC0
                slot = jj & 1
                cps = w13_copies(j, w13_r.at[slot], SEM_W + 4 * slot)
                for cp in (cps[:2] if MIDWAIT else cps):
                    cp.wait()

                def mid():
                    for cp in cps[2:]:
                        cp.wait()
                for pp in range(3):
                    @pl.when(jj == 4 * pp)
                    def _():
                        wqkv_copy(pp).wait()

                @pl.when(jj + 1 < NMAIN)
                def _():
                    for cp in w13_copies(j + 1, w13_r.at[1 - slot], SEM_W + 4 * (1 - slot)):
                        cp.start()

                if QPOS == 0:
                    qkv_tile(jj >> 2, jj & 3)
                ops = gate_up2(w13_r.at[slot])
                if QPOS == 1:
                    qkv_tile(jj >> 2, jj & 3)
                for a in range(2):
                    for t in range(7):
                        hl[j, t, a * (QS // 2):(a + 1) * (QS // 2), :] = ops[a][t]
                if QPOS == 2:
                    qkv_tile(jj >> 2, jj & 3)
                return carry

            with scope("P_main"):
                lax.fori_loop(0, NMAIN, main_body, 0)

        def phase_b(ol, b_v, out_v, wo_t):
            def attn_rows(r, masked, tok, never):
                ln = lax.broadcasted_iota(jnp.int32, (8, 128), 1)
                row = lax.broadcasted_iota(jnp.int32, (8, 128), 0) * 2 + r
                q = [qkv[j, pl.ds(r + PAD, 8, stride=2), :] for j in range(8)]
                if tok is not None:
                    q = [jnp.where(never, tok, qq) if j < GATE else qq for j, qq in enumerate(q)]
                logits = []
                for w in range(WIN):
                    p = None
                    for j in range(8):
                        t = q[j] * qkv[8 + j, pl.ds(r + (PAD - DIL * w), 8, stride=2), :]
                        p = t if p is None else p + t
                    p = p + pltpu.roll(p, 64, 1)
                    p = p + jnp.take_along_axis(p, ln ^ 1, axis=1)
                    if w > 0 and masked:
                        p = jnp.where(row >= DIL * w, p, MASKED)
                    logits.append(p)
                mx = logits[0]
                for w in range(1, WIN):
                    mx = jnp.maximum(mx, logits[w])
                es = [jnp.exp2(l - mx) for l in logits]
                den = es[0]
                for w in range(1, WIN):
                    den = den + es[w]
                inv = 1.0 / den
                outs = []
                for j in range(8):
                    o = None
                    for w in range(WIN):
                        t = es[w] * qkv[16 + j, pl.ds(r + (PAD - DIL * w), 8, stride=2), :]
                        o = t if o is None else o + t
                    outs.append(o * inv)
                return outs

            def attn_group(r, rh, masked, tok, never):
                res = []
                for hf in range(2):
                    pair = []
                    for e in range(2):
                        pair.append(attn_rows(hf * HS + r + e, masked and hf == 0, tok, never))
                        if CHAIN == 1 or (CHAIN == 2 and e == 1) or (CHAIN == 4 and e == 1 and hf == 1):
                            tok = pair[-1][7]
                    res.append(pair)
                top, bot = res
                for j in range(4):
                    ops = _lhs_words(*[(v[0][c], v[1][c]) for v, c in ((top, j), (top, 4 + j), (bot, j), (bot, 4 + j))])
                    for t in range(7):
                        ol[t, pl.ds(rh, 8), j * 128:(j + 1) * 128] = ops[t]
                return tok

            def down_body(n, carry):
                def wot():
                    wo_t[n] = pltpu.bitcast(wo_r[n], jnp.uint32)
                    wo_t[4 + n] = pltpu.bitcast(wo_r[4 + n], jnp.uint32)
                if WOT == 0:
                    wot()
                a0h = pl.multiple_of(n * (AT_ROWS // 2), AT_ROWS // 2)
                a0 = pl.multiple_of(n * AT_ROWS, AT_ROWS)

                def attention():
                    tok = None
                    never = lax.broadcasted_iota(jnp.int32, (8, 128), 1) < (n - 1048576)
                    for g in range(AT_ROWS // 16):
                        tok = attn_group(a0 + g * 16, a0h + g * 8, g == 0, tok, never)
                if ATPOS == 0:
                    attention()
                rhs = _rhs_combos(w2_r[n, 0:HF, :], w2_r[4 + n, 0:HF, :], w2_r[n, HF:F, :], w2_r[4 + n, HF:F, :])
                lhs = lambda t: jnp.concatenate([_unpk(hl[j, t]) for j in range(NCH)], axis=1)
                c11, c12, c21, c22 = _out_combos(_products(lhs, rhs, DORDER))
                b_v[n, 0:HS, :] = c11
                b_v[4 + n, 0:HS, :] = c12
                b_v[n, HS:S, :] = c21
                b_v[4 + n, HS:S, :] = c22
                if ATPOS == 1:
                    attention()
                if WOT == 1:
                    wot()
                return carry

            with scope("P_down"):
                for n in range(8):
                    w2_copy(n).wait()
                    wo_copy(n).wait()
                lax.fori_loop(0, 4, down_body, 0)

            def out_copy(tile, half):
                c = pl.multiple_of(tile * 128, 128)
                return pltpu.make_async_copy(out_v.at[tile, pl.ds(half * HS, HS)],
                                             out_hbm.at[pl.ds(half * HS, HS), pl.ds(c, 128)], osem.at[tile * 2 + half])

            def fin_body(n, carry):
                def rows(tile, lo):
                    parts = [wo_t[tile, pl.ds(dd, 32, stride=16), :] for dd in range(lo, lo + 8)]
                    return jnp.concatenate(parts, axis=0)
                rhs = [_unpk(v) for v in _rhs_words(rows(n, 0), rows(4 + n, 0), rows(n, 8), rows(4 + n, 8))]
                s_q = _out_combos(_products(lambda t: _unpk(ol[t]), rhs, FORDER))
                quads = ((n, 0), (4 + n, 0), (n, 1), (4 + n, 1))
                for k in (1, 2, 3, 0):
                    tile, half = quads[k]
                    c = pl.multiple_of(tile * 128, 128)
                    rs = pl.ds(half * HS, HS)
                    g = _silu(b_v[tile, rs, :])
                    out_v[tile, rs, :] = (x_v[rs, pl.ds(c, 128)].astype(F32) + s_q[k] * g).astype(BF16)
                    out_copy(tile, half).start()
                return carry

            with scope("P_fin"):
                lax.fori_loop(0, 4, fin_body, 0)
                for tile in range(8):
                    for half in range(2):
                        out_copy(tile, half).wait()

        pl.run_scoped(phase_a, *scoped_a)
        pl.run_scoped(phase_b, *scoped_b)

    scoped_a = [
        pltpu.VMEM((7, HS // 2, HD), jnp.uint32),
        pltpu.VMEM((49, S // 8, QD), jnp.uint32),
        pltpu.VMEM((NC0, 2, 7, HD // 2, 128), jnp.uint32),
        pltpu.VMEM((8, S // 4, 128), F32),
        pltpu.VMEM((3, D, D), BF16),
        pltpu.VMEM((NC0, 4, D, 128), BF16),
        pltpu.VMEM((2, 4, D, 128), BF16),
    ]
    scoped_b = [
        pltpu.VMEM((7, HS // 2, HD), jnp.uint32),
        pltpu.VMEM((8, S, 128), F32),
        pltpu.VMEM((8, S, 128), BF16),
        pltpu.VMEM((8, D // 2, 128), jnp.uint32),
    ]
    scratch = [
        pltpu.VMEM((S, D), BF16),
        pltpu.VMEM((8, F, 128), BF16),
        pltpu.VMEM((8, D, 128), BF16),
        pltpu.VMEM((NCH, 7, HS // 2, 128), jnp.uint32),
        pltpu.VMEM((24, S + PAD, 128), F32),
        pltpu.SemaphoreType.DMA((4 * NRP + 3 + 4 * NC0 + 24,)),
        pltpu.SemaphoreType.DMA((16,)),
    ]
    return kernel, scratch


_CFG = dict(LG=64)


@jax.jit
def pallas_recurrent_scan__sliding_local_dilated__glu_gated_swiglu__prompt_kernel(
    A_x: jax.Array,
    A_wqkv: jax.Array,
    A_wo: jax.Array,
    B_x: jax.Array,
    B_w1: jax.Array,
    B_w3: jax.Array,
    B_w2: jax.Array,
):
    del B_x
    kernel, scratch = make_kernel(**_CFG)
    any_spec = pl.BlockSpec(memory_space=pl.ANY)
    out = pl.pallas_call(
        kernel,
        out_shape=jax.ShapeDtypeStruct((S, D), BF16),
        in_specs=[any_spec] * 6,
        out_specs=any_spec,
        scratch_shapes=scratch,
        compiler_params=pltpu.CompilerParams(
            vmem_limit_bytes=120 * 2**20,
            flags={"XLA_TPU_EVENLY_DISTRIBUTE_CRITICAL_NODES": True},
        ),
    )(A_x.reshape(S, D), A_wqkv, A_wo, B_w1, B_w3, B_w2)
    return out.reshape(1, S, D)
```

```python
import jax
import jax.numpy as jnp
import numpy as np
from jax import lax
import jax.experimental.pallas as pl
import jax.experimental.pallas.tpu as pltpu

S, D, F = 2048, 1024, 3584
H, DH, WIN, DIL = 32, 32, 8, 2
HS = S // 2
HD = D // 2
QD = D // 4
HF = F // 2
NCH = HF // 128
F32, BF16 = jnp.float32, jnp.bfloat16
EPS = 1e-5
SCALE = DH ** -0.5
LOG2E = 1.4426950408889634
MASKED = -1e9 * LOG2E
ORDER = (1, 4, 0, 2, 3, 5, 6)
INNER_ORDER = (4, 1, 2, 3, 0, 5, 6)
PAD = 16


def _dot(a, b):
    return jnp.dot(a, b, preferred_element_type=F32)


def _lhs_combos(a11, a12, a21, a22):
    return [a11 + a22, a21 + a22, a11, a22, a11 + a12, a21 - a11, a12 - a22]


def _rhs_combos(b11, b12, b21, b22):
    return [_unpk(v) for v in _rhs_words(*[_words(b) for b in (b11, b12, b21, b22)])]


def _lin_combos(b11, b12, b21, b22):
    return [b11 + b22, b11, b12 - b22, b21 - b11, b22, b11 + b12, b21 + b22]


def _eo(w):
    return (pltpu.bitcast(w << 16, F32), pltpu.bitcast(w & np.uint32(0xFFFF0000), F32))


def _pk_eo(e, o):
    return pltpu.pack_elementwise([e, o], packed_dtype=BF16)


def _words(x):
    return pltpu.bitcast(x, jnp.uint32)


def _rhs_words(b11, b12, b21, b22):
    eo = [_eo(b) for b in (b11, b12, b21, b22)]
    ce = _lin_combos(*[v[0] for v in eo])
    co = _lin_combos(*[v[1] for v in eo])
    return [b11 if t == 1 else b22 if t == 4 else _pk_eo(ce[t], co[t]) for t in range(7)]


def _lhs_words(a11, a12, a21, a22):
    ce = _lhs_combos(a11[0], a12[0], a21[0], a22[0])
    co = _lhs_combos(a11[1], a12[1], a21[1], a22[1])
    return [_pk_eo(e, o) for e, o in zip(ce, co)]


def _products(lhs, rhs, order):
    m = [None] * 7
    for t in order:
        m[t] = _dot(lhs(t), rhs[t])
    return m


def _out_combos(m):
    m1, m2, m3, m4, m5, m6, m7 = m
    c11 = (m1 + m4) + (m7 - m5)
    c12 = m3 + m5
    c21 = m2 + m4
    c22 = (m1 + m3) + (m6 - m2)
    return c11, c12, c21, c22


def _pk(x):
    return pltpu.bitcast(x.astype(BF16), jnp.uint32)


def _unpk(x):
    return pltpu.bitcast(x, BF16)


def _silu(x):
    hx = 0.5 * x
    return hx + hx * jnp.tanh(hx)


def _make_kernel():
    RQ = 128
    LG = 64
    NC0 = 2
    QS = S // 4
    NRP = QS // RQ
    NMAIN = NCH - NC0
    AT_ROWS = HS // 4

    def kernel(x_hbm, wqkv_hbm, wo_hbm, w1_hbm, w3_hbm, w2_hbm, out_hbm,
               x_v, w2_r, wo_r, hl, qkv, sems, osem):
        SB = 4 * NRP
        SEM_W0 = SB + 3
        SEM_W = SEM_W0 + 4 * NC0
        SEM_W2 = SEM_W + 8
        SEM_WO = SEM_W2 + 8

        def w2_copy(n):
            return pltpu.make_async_copy(w2_hbm.at[:, pl.ds(n * 128, 128)], w2_r.at[n], sems.at[SEM_W2 + n])

        def wo_copy(n):
            return pltpu.make_async_copy(wo_hbm.at[:, pl.ds(n * 128, 128)], wo_r.at[n], sems.at[SEM_WO + n])

        def phase_a(xl, xl2, rg, wqkv_r, w13_0, w13_r):
            def x_copy(i, q):
                r = q * QS + i * RQ
                return pltpu.make_async_copy(x_hbm.at[pl.ds(r, RQ)], x_v.at[pl.ds(r, RQ)], sems.at[q * NRP + i])

            def wqkv_copy(p):
                return pltpu.make_async_copy(wqkv_hbm.at[:, pl.ds(p * D, D)], wqkv_r.at[p], sems.at[SB + p])

            def w13_copies(j, dst, sem0):
                c = pl.multiple_of(j * 128, 128)
                return [
                    pltpu.make_async_copy(w1_hbm.at[:, pl.ds(c, 128)], dst.at[0], sems.at[sem0]),
                    pltpu.make_async_copy(w3_hbm.at[:, pl.ds(c, 128)], dst.at[2], sems.at[sem0 + 1]),
                    pltpu.make_async_copy(w1_hbm.at[:, pl.ds(HF + c, 128)], dst.at[1], sems.at[sem0 + 2]),
                    pltpu.make_async_copy(w3_hbm.at[:, pl.ds(HF + c, 128)], dst.at[3], sems.at[sem0 + 3]),
                ]

            def ln_rows(r, n):
                outs = []
                for xv in _eo(_words(x_v[pl.ds(r, n), :])):
                    mean = jnp.sum(xv, axis=-1, keepdims=True) * (1.0 / D)
                    xc = xv - mean
                    var = jnp.sum(xc * xc, axis=-1, keepdims=True) * (1.0 / D)
                    outs.append(xc * lax.rsqrt(var + EPS))
                return outs

            def ln_vals(r, two=True):
                p1a, p1b = [[] for _ in range(7)], [[] for _ in range(7)]
                p2 = [[] for _ in range(49)]
                for g in range(0, RQ, LG):
                    rows = [ln_rows(q * QS + r + g, LG) for q in range(4)]
                    la, lb = [], []
                    for e in range(2):
                        rw = [v[e] for v in rows]
                        la.append(_lhs_combos(rw[0][:, :HD], rw[0][:, HD:], rw[2][:, :HD], rw[2][:, HD:]))
                        lb.append(_lhs_combos(rw[1][:, :HD], rw[1][:, HD:], rw[3][:, :HD], rw[3][:, HD:]))
                    for t in range(7):
                        p1a[t].append(_pk_eo(la[0][t], la[1][t]))
                        p1b[t].append(_pk_eo(lb[0][t], lb[1][t]))
                        if two:
                            inner = [_lhs_combos(la[e][t][:, :QD], la[e][t][:, QD:], lb[e][t][:, :QD], lb[e][t][:, QD:])
                                     for e in range(2)]
                            for u in range(7):
                                p2[t * 7 + u].append(_pk_eo(inner[0][u], inner[1][u]))
                cat = lambda ps: [jnp.concatenate(p, axis=0) if len(p) > 1 else p[0] for p in ps]
                return cat(p1a), cat(p1b), cat(p2) if two else []

            def ln_store(rh, vals):
                va, vb, v2 = vals
                for t in range(7):
                    xl[t, pl.ds(rh, RQ // 2), :] = va[t]
                    xl[t, pl.ds(QS // 2 + rh, RQ // 2), :] = vb[t]
                for t in range(len(v2)):
                    xl2[t, pl.ds(rh, RQ // 2), :] = v2[t]

            def first_rhs(w, half):
                w1, w3 = w.at[half], w.at[2 + half]
                return _rhs_words(*[_words(v) for v in (w1[0:HD, :], w3[0:HD, :], w1[HD:D, :], w3[HD:D, :])])

            def gate_up(lhs, c0):
                hs = []
                for half in range(2):
                    rhs = [_unpk(rg[c0, half, t]) for t in range(7)]
                    g_top, u_top, g_bot, u_bot = _out_combos(_products(lhs, rhs, ORDER))
                    hs.append((_silu(g_top) * u_top, _silu(g_bot) * u_bot))
                return [_pk(v) for v in _lhs_combos(hs[0][0], hs[1][0], hs[0][1], hs[1][1])]

            def gate_up2(w):
                blk = lambda kq, nq: _eo(_words(w[nq, kq * QD:(kq + 1) * QD, :]))
                big = [[[[blk(2 * kh + a, 2 * nh + b) for b in range(2)] for a in range(2)] for nh in range(2)] for kh in range(2)]
                mm = [None] * 7
                for t in ORDER:
                    inner = []
                    for e in range(2):
                        r = [[_lin_combos(big[0][0][a][b][e], big[0][1][a][b][e], big[1][0][a][b][e], big[1][1][a][b][e])[t]
                              for b in range(2)] for a in range(2)]
                        inner.append(_lin_combos(r[0][0], r[0][1], r[1][0], r[1][1]))
                    rr = [_unpk(_pk_eo(ve, vo)) for ve, vo in zip(*inner)]
                    c = _out_combos(_products(lambda u: _unpk(xl2[t * 7 + u]), rr, INNER_ORDER))
                    mm[t] = [[c[0], c[1]], [c[2], c[3]]]
                cc = [[None] * 4 for _ in range(4)]
                for a in range(2):
                    for b in range(2):
                        o11, o12, o21, o22 = _out_combos([mm[t][a][b] for t in range(7)])
                        cc[a][b], cc[a][2 + b], cc[2 + a][b], cc[2 + a][2 + b] = o11, o12, o21, o22
                h = [[_silu(cc[q][b]) * cc[q][2 + b] for b in range(2)] for q in range(4)]
                return [[_pk(v) for v in _lhs_combos(h[a][0], h[a][1], h[2 + a][0], h[2 + a][1])] for a in range(2)]

            for q in range(4):
                x_copy(0, q).start()
            for c0 in range(NC0):
                for cp in w13_copies(c0, w13_0.at[c0], SEM_W0 + 4 * c0):
                    cp.start()
            for j in range(8, 24):
                qkv[j, 0:PAD, :] = jnp.zeros((PAD, 128), F32)
            for q in range(4):
                x_copy(0, q).wait()
            for i in range(1, NRP):
                for q in range(4):
                    x_copy(i, q).start()
            ln_store(0, ln_vals(0, False))
            for c0 in range(NC0):
                for cp in w13_copies(c0, w13_0.at[c0], SEM_W0 + 4 * c0):
                    cp.wait()
                for half in range(2):
                    rhs = first_rhs(w13_0.at[c0], half)
                    for t in range(7):
                        rg[c0, half, t] = rhs[t]
            for cp in w13_copies(NC0, w13_r.at[0], SEM_W):
                cp.start()
            for p in range(3):
                wqkv_copy(p).start()
            for n in range(8):
                w2_copy(n).start()
            for n in range(8):
                wo_copy(n).start()

            def first_body(i, carry):
                for ii in range(1, NRP):
                    @pl.when(i + 1 == ii)
                    def _():
                        for q in range(4):
                            x_copy(ii, q).wait()
                inext = jnp.where(i + 1 == NRP, 0, i + 1)
                rn = pl.multiple_of(inext * RQ, RQ)
                rh = pl.multiple_of(i * (RQ // 2), RQ // 2)
                rnh = pl.multiple_of(inext * (RQ // 2), RQ // 2)
                lhs_vals = [_unpk(jnp.concatenate([xl[t, pl.ds(rh, RQ // 2), :], xl[t, pl.ds(QS // 2 + rh, RQ // 2), :]], axis=0))
                            for t in range(7)]
                nxt = ln_vals(rn)
                for c0 in range(NC0):
                    ops = gate_up(lambda t: lhs_vals[t], c0)
                    for t in range(7):
                        pk = ops[t]
                        hl[c0, t, pl.ds(rh, RQ // 2), :] = pk[0:RQ // 2]
                        hl[c0, t, pl.ds(QS // 2 + rh, RQ // 2), :] = pk[RQ // 2:RQ]
                ln_store(rnh, nxt)
                return carry

            lax.fori_loop(0, NRP, first_body, 0)

            def qkv_tile(p, i):
                ln = lax.broadcasted_iota(jnp.int32, (D // 2, 128), 1)
                pos = (ln >> 2) & 7
                ys = []
                for j in range(8):
                    v = pltpu.bitcast(wqkv_r[p, :, j * 128:(j + 1) * 128], jnp.uint32)
                    ys.append(v if j == 0 else pltpu.roll(v, 4 * j, 1))
                hh_full = (ln >> 1) & 31
                base = ((hh_full & 3) * 8 + (hh_full >> 2))
                low = (ln >> 6) * 2 + (ln & 1)

                def column_tile(ii):
                    sel = (pos - ii) & 7
                    z = ys[0]
                    for j in range(1, 8):
                        z = jnp.where(sel == j, ys[j], z)
                    src = (((base + ii) & 31) << 2) + low
                    return jnp.take_along_axis(z, src, axis=1)

                left = column_tile(i)
                right = column_tile(i + 4)
                rhs = [_unpk(v) for v in _rhs_words(left[:QD], right[:QD], left[QD:], right[QD:])]
                c11, c12, c21, c22 = _out_combos(_products(lambda t: _unpk(xl[t]), rhs, ORDER))
                sc = jnp.where(p == 0, SCALE * LOG2E, 1.0).astype(F32)
                c11, c12, c21, c22 = c11 * sc, c12 * sc, c21 * sc, c22 * sc
                qkv[p * 8 + i, PAD:PAD + HS, :] = c11
                qkv[p * 8 + 4 + i, PAD:PAD + HS, :] = c12
                qkv[p * 8 + i, PAD + HS:PAD + S, :] = c21
                qkv[p * 8 + 4 + i, PAD + HS:PAD + S, :] = c22

            def main_body(jj, carry):
                j = jj + NC0
                slot = jj & 1
                for cp in w13_copies(j, w13_r.at[slot], SEM_W + 4 * slot):
                    cp.wait()
                for pp in range(3):
                    @pl.when(jj == 4 * pp)
                    def _():
                        wqkv_copy(pp).wait()

                @pl.when(jj + 1 < NMAIN)
                def _():
                    for cp in w13_copies(j + 1, w13_r.at[1 - slot], SEM_W + 4 * (1 - slot)):
                        cp.start()

                ops = gate_up2(w13_r.at[slot])
                for a in range(2):
                    for t in range(7):
                        hl[j, t, a * (QS // 2):(a + 1) * (QS // 2), :] = ops[a][t]
                qkv_tile(jj >> 2, jj & 3)
                return carry

            lax.fori_loop(0, NMAIN, main_body, 0)

        def phase_b(ol, b_v, out_v, wo_t):
            def attn_rows(r, masked, tok, never):
                ln = lax.broadcasted_iota(jnp.int32, (8, 128), 1)
                row = lax.broadcasted_iota(jnp.int32, (8, 128), 0) * 2 + r
                q = [qkv[j, pl.ds(r + PAD, 8, stride=2), :] for j in range(8)]
                if tok is not None:
                    q = [jnp.where(never, tok, qq) for qq in q]
                logits = []
                for w in range(WIN):
                    p = None
                    for j in range(8):
                        t = q[j] * qkv[8 + j, pl.ds(r + (PAD - DIL * w), 8, stride=2), :]
                        p = t if p is None else p + t
                    p = p + pltpu.roll(p, 64, 1)
                    p = p + jnp.take_along_axis(p, ln ^ 1, axis=1)
                    if w > 0 and masked:
                        p = jnp.where(row >= DIL * w, p, MASKED)
                    logits.append(p)
                mx = logits[0]
                for w in range(1, WIN):
                    mx = jnp.maximum(mx, logits[w])
                es = [jnp.exp2(l - mx) for l in logits]
                den = es[0]
                for w in range(1, WIN):
                    den = den + es[w]
                inv = 1.0 / den
                outs = []
                for j in range(8):
                    o = None
                    for w in range(WIN):
                        t = es[w] * qkv[16 + j, pl.ds(r + (PAD - DIL * w), 8, stride=2), :]
                        o = t if o is None else o + t
                    outs.append(o * inv)
                return outs

            def attn_group(r, rh, masked, tok, never):
                res = []
                for hf in range(2):
                    pair = []
                    for e in range(2):
                        pair.append(attn_rows(hf * HS + r + e, masked and hf == 0, tok, never))
                    res.append(pair)
                tok = res[1][1][7]
                top, bot = res
                for j in range(4):
                    ops = _lhs_words(*[(v[0][c], v[1][c]) for v, c in ((top, j), (top, 4 + j), (bot, j), (bot, 4 + j))])
                    for t in range(7):
                        ol[t, pl.ds(rh, 8), j * 128:(j + 1) * 128] = ops[t]
                return tok

            def down_body(n, carry):
                wo_t[n, 0:HD, :] = _words(wo_r[n])
                wo_t[4 + n, 0:HD, :] = _words(wo_r[4 + n])
                a0h = pl.multiple_of(n * (AT_ROWS // 2), AT_ROWS // 2)
                a0 = pl.multiple_of(n * AT_ROWS, AT_ROWS)

                tok = None
                never = lax.broadcasted_iota(jnp.int32, (8, 128), 1) < (n - 1048576)
                for g in range(AT_ROWS // 16):
                    tok = attn_group(a0 + g * 16, a0h + g * 8, g == 0, tok, never)
                rhs = _rhs_combos(w2_r[n, 0:HF, :], w2_r[4 + n, 0:HF, :], w2_r[n, HF:F, :], w2_r[4 + n, HF:F, :])
                lhs = lambda t: jnp.concatenate([_unpk(hl[j, t]) for j in range(NCH)], axis=1)
                c11, c12, c21, c22 = _out_combos(_products(lhs, rhs, ORDER))
                b_v[n, 0:HS, :] = c11
                b_v[4 + n, 0:HS, :] = c12
                b_v[n, HS:S, :] = c21
                b_v[4 + n, HS:S, :] = c22
                return carry

            for n in range(8):
                w2_copy(n).wait()
                wo_copy(n).wait()
            lax.fori_loop(0, 4, down_body, 0)

            def out_copy(tile, half):
                c = pl.multiple_of(tile * 128, 128)
                return pltpu.make_async_copy(out_v.at[tile, pl.ds(half * HS, HS)],
                                             out_hbm.at[pl.ds(half * HS, HS), pl.ds(c, 128)], osem.at[tile * 2 + half])

            def fin_body(n, carry):
                def rows(tile, lo):
                    parts = [wo_t[tile, pl.ds(dd, 32, stride=16), :] for dd in range(lo, lo + 8)]
                    return jnp.concatenate(parts, axis=0)
                rhs = [_unpk(v) for v in _rhs_words(rows(n, 0), rows(4 + n, 0), rows(n, 8), rows(4 + n, 8))]
                s_q = _out_combos(_products(lambda t: _unpk(ol[t]), rhs, ORDER))
                quads = ((n, 0), (4 + n, 0), (n, 1), (4 + n, 1))
                for k in (1, 2, 3, 0):
                    tile, half = quads[k]
                    c = pl.multiple_of(tile * 128, 128)
                    rs = pl.ds(half * HS, HS)
                    g = _silu(b_v[tile, rs, :])
                    out_v[tile, rs, :] = (x_v[rs, pl.ds(c, 128)].astype(F32) + s_q[k] * g).astype(BF16)
                    out_copy(tile, half).start()
                return carry

            lax.fori_loop(0, 4, fin_body, 0)
            for tile in range(8):
                for half in range(2):
                    out_copy(tile, half).wait()

        pl.run_scoped(phase_a, *scoped_a)
        pl.run_scoped(phase_b, *scoped_b)

    scoped_a = [
        pltpu.VMEM((7, HS // 2, HD), jnp.uint32),
        pltpu.VMEM((49, S // 8, QD), jnp.uint32),
        pltpu.VMEM((NC0, 2, 7, HD // 2, 128), jnp.uint32),
        pltpu.VMEM((3, D, D), BF16),
        pltpu.VMEM((NC0, 4, D, 128), BF16),
        pltpu.VMEM((2, 4, D, 128), BF16),
    ]
    scoped_b = [
        pltpu.VMEM((7, HS // 2, HD), jnp.uint32),
        pltpu.VMEM((8, S, 128), F32),
        pltpu.VMEM((8, S, 128), BF16),
        pltpu.VMEM((8, D // 2 + 16, 128), jnp.uint32),
    ]
    scratch = [
        pltpu.VMEM((S, D), BF16),
        pltpu.VMEM((8, F, 128), BF16),
        pltpu.VMEM((8, D, 128), BF16),
        pltpu.VMEM((NCH, 7, HS // 2, 128), jnp.uint32),
        pltpu.VMEM((24, S + 5 * PAD, 128), F32),
        pltpu.SemaphoreType.DMA((4 * NRP + 3 + 4 * NC0 + 24,)),
        pltpu.SemaphoreType.DMA((16,)),
    ]
    return kernel, scratch


@jax.jit
def pallas_recurrent_scan__sliding_local_dilated__glu_gated_swiglu__prompt_kernel(
    A_x: jax.Array,
    A_wqkv: jax.Array,
    A_wo: jax.Array,
    B_x: jax.Array,
    B_w1: jax.Array,
    B_w3: jax.Array,
    B_w2: jax.Array,
):
    del B_x
    kernel, scratch = _make_kernel()
    any_spec = pl.BlockSpec(memory_space=pl.ANY)
    out = pl.pallas_call(
        kernel,
        out_shape=jax.ShapeDtypeStruct((S, D), BF16),
        in_specs=[any_spec] * 6,
        out_specs=any_spec,
        scratch_shapes=scratch,
        compiler_params=pltpu.CompilerParams(
            vmem_limit_bytes=120 * 2**20,
            flags={"XLA_TPU_EVENLY_DISTRIBUTE_CRITICAL_NODES": True},
        ),
    )(A_x.reshape(S, D), A_wqkv, A_wo, B_w1, B_w3, B_w2)
    return out.reshape(1, S, D)
```

```python
import jax
import jax.numpy as jnp
from jax import lax
import jax.experimental.pallas as pl
import jax.experimental.pallas.tpu as pltpu

S, D, F = 2048, 1024, 3584
H, DH, WIN, DIL = 32, 32, 8, 2
HS = S // 2
HD = D // 2
QD = D // 4
HF = F // 2
NCH = HF // 128
F32, BF16 = jnp.float32, jnp.bfloat16
EPS = 1e-5
SCALE = DH ** -0.5
LOG2E = 1.4426950408889634
MASKED = -1e9 * LOG2E
ORDER = (1, 4, 0, 2, 3, 5, 6)
INNER_ORDER = (4, 1, 2, 3, 0, 5, 6)
PAD = 16


def _dot(a, b):
    return jnp.dot(a, b, preferred_element_type=F32)


def _lhs_combos(a11, a12, a21, a22):
    return [a11 + a22, a21 + a22, a11, a22, a11 + a12, a21 - a11, a12 - a22]


def _rhs_combos(b11, b12, b21, b22):
    return [_unpk(v) for v in _rhs_words(*[_words(b) for b in (b11, b12, b21, b22)])]


def _lin_combos(b11, b12, b21, b22):
    return [b11 + b22, b11, b12 - b22, b21 - b11, b22, b11 + b12, b21 + b22]


def _eo(w):
    v = _unpk(w).astype(F32)
    n = w.shape[0]
    return v[0:n], v[n:2 * n]


def _pk_eo(e, o):
    return _pk(jnp.concatenate([e, o], axis=0))


def _words(x):
    return pltpu.bitcast(x, jnp.uint32)


def _rhs_words(b11, b12, b21, b22):
    eo = [_eo(b) for b in (b11, b12, b21, b22)]
    ce = _lin_combos(*[v[0] for v in eo])
    co = _lin_combos(*[v[1] for v in eo])
    return [b11 if t == 1 else b22 if t == 4 else _pk_eo(ce[t], co[t]) for t in range(7)]


def _lhs_words(a11, a12, a21, a22):
    ce = _lhs_combos(a11[0], a12[0], a21[0], a22[0])
    co = _lhs_combos(a11[1], a12[1], a21[1], a22[1])
    return [_pk_eo(e, o) for e, o in zip(ce, co)]


def _products(lhs, rhs, order):
    m = [None] * 7
    for t in order:
        m[t] = _dot(lhs(t), rhs[t])
    return m


def _out_combos(m):
    m1, m2, m3, m4, m5, m6, m7 = m
    c11 = (m1 + m4) + (m7 - m5)
    c12 = m3 + m5
    c21 = m2 + m4
    c22 = (m1 + m3) + (m6 - m2)
    return c11, c12, c21, c22


def _pk(x):
    return pltpu.bitcast(x.astype(BF16), jnp.uint32)


def _unpk(x):
    return pltpu.bitcast(x, BF16)


def _silu(x):
    hx = 0.5 * x
    return hx + hx * jnp.tanh(hx)


def _make_kernel():
    RQ = 128
    LG = 64
    NC0 = 2
    QS = S // 4
    NRP = QS // RQ
    NMAIN = NCH - NC0
    AT_ROWS = HS // 4

    def kernel(x_hbm, wqkv_hbm, wo_hbm, w1_hbm, w3_hbm, w2_hbm, out_hbm,
               x_v, w2_r, wo_r, hl, qkv, sems, osem):
        SB = 4 * NRP
        SEM_W0 = SB + 3
        SEM_W = SEM_W0 + 4 * NC0
        SEM_W2 = SEM_W + 8
        SEM_WO = SEM_W2 + 8

        def w2_copy(n):
            return pltpu.make_async_copy(w2_hbm.at[:, pl.ds(n * 128, 128)], w2_r.at[n], sems.at[SEM_W2 + n])

        def wo_copy(n):
            return pltpu.make_async_copy(wo_hbm.at[:, pl.ds(n * 128, 128)], wo_r.at[n], sems.at[SEM_WO + n])

        def phase_a(xl, xl2, rg, wqkv_r, w13_0, w13_r):
            def x_copy(i, q):
                r = q * QS + i * RQ
                return pltpu.make_async_copy(x_hbm.at[pl.ds(r, RQ)], x_v.at[pl.ds(r, RQ)], sems.at[q * NRP + i])

            def wqkv_copy(p):
                return pltpu.make_async_copy(wqkv_hbm.at[:, pl.ds(p * D, D)], wqkv_r.at[p], sems.at[SB + p])

            def w13_copies(j, dst, sem0):
                c = pl.multiple_of(j * 128, 128)
                return [
                    pltpu.make_async_copy(w1_hbm.at[:, pl.ds(c, 128)], dst.at[0], sems.at[sem0]),
                    pltpu.make_async_copy(w3_hbm.at[:, pl.ds(c, 128)], dst.at[2], sems.at[sem0 + 1]),
                    pltpu.make_async_copy(w1_hbm.at[:, pl.ds(HF + c, 128)], dst.at[1], sems.at[sem0 + 2]),
                    pltpu.make_async_copy(w3_hbm.at[:, pl.ds(HF + c, 128)], dst.at[3], sems.at[sem0 + 3]),
                ]

            def ln_rows(r, n):
                outs = []
                for xv in _eo(_words(x_v[pl.ds(r, n), :])):
                    mean = jnp.sum(xv, axis=-1, keepdims=True) * (1.0 / D)
                    xc = xv - mean
                    var = jnp.sum(xc * xc, axis=-1, keepdims=True) * (1.0 / D)
                    outs.append(xc * lax.rsqrt(var + EPS))
                return outs

            def ln_vals(r, two=True):
                p1a, p1b = [[] for _ in range(7)], [[] for _ in range(7)]
                p2 = [[] for _ in range(49)]
                for g in range(0, RQ, LG):
                    rows = [ln_rows(q * QS + r + g, LG) for q in range(4)]
                    la, lb = [], []
                    for e in range(2):
                        rw = [v[e] for v in rows]
                        la.append(_lhs_combos(rw[0][:, :HD], rw[0][:, HD:], rw[2][:, :HD], rw[2][:, HD:]))
                        lb.append(_lhs_combos(rw[1][:, :HD], rw[1][:, HD:], rw[3][:, :HD], rw[3][:, HD:]))
                    for t in range(7):
                        p1a[t].append(_pk_eo(la[0][t], la[1][t]))
                        p1b[t].append(_pk_eo(lb[0][t], lb[1][t]))
                        if two:
                            inner = [_lhs_combos(la[e][t][:, :QD], la[e][t][:, QD:], lb[e][t][:, :QD], lb[e][t][:, QD:])
                                     for e in range(2)]
                            for u in range(7):
                                p2[t * 7 + u].append(_pk_eo(inner[0][u], inner[1][u]))
                cat = lambda ps: [jnp.concatenate(p, axis=0) if len(p) > 1 else p[0] for p in ps]
                return cat(p1a), cat(p1b), cat(p2) if two else []

            def ln_store(rh, vals):
                va, vb, v2 = vals
                for t in range(7):
                    xl[t, pl.ds(rh, RQ // 2), :] = va[t]
                    xl[t, pl.ds(QS // 2 + rh, RQ // 2), :] = vb[t]
                for t in range(len(v2)):
                    xl2[t, pl.ds(rh, RQ // 2), :] = v2[t]

            def first_rhs(w, half):
                w1, w3 = w.at[half], w.at[2 + half]
                return _rhs_words(*[_words(v) for v in (w1[0:HD, :], w3[0:HD, :], w1[HD:D, :], w3[HD:D, :])])

            def gate_up(lhs, c0):
                hs = []
                for half in range(2):
                    rhs = [_unpk(rg[c0, half, t]) for t in range(7)]
                    g_top, u_top, g_bot, u_bot = _out_combos(_products(lhs, rhs, ORDER))
                    hs.append((_silu(g_top) * u_top, _silu(g_bot) * u_bot))
                return [_pk(v) for v in _lhs_combos(hs[0][0], hs[1][0], hs[0][1], hs[1][1])]

            def gate_up2(w):
                blk = lambda kq, nq: _eo(_words(w[nq, kq * QD:(kq + 1) * QD, :]))
                big = [[[[blk(2 * kh + a, 2 * nh + b) for b in range(2)] for a in range(2)] for nh in range(2)] for kh in range(2)]
                mm = [None] * 7
                for t in ORDER:
                    inner = []
                    for e in range(2):
                        r = [[_lin_combos(big[0][0][a][b][e], big[0][1][a][b][e], big[1][0][a][b][e], big[1][1][a][b][e])[t]
                              for b in range(2)] for a in range(2)]
                        inner.append(_lin_combos(r[0][0], r[0][1], r[1][0], r[1][1]))
                    rr = [_unpk(_pk_eo(ve, vo)) for ve, vo in zip(*inner)]
                    c = _out_combos(_products(lambda u: _unpk(xl2[t * 7 + u]), rr, INNER_ORDER))
                    mm[t] = [[c[0], c[1]], [c[2], c[3]]]
                cc = [[None] * 4 for _ in range(4)]
                for a in range(2):
                    for b in range(2):
                        o11, o12, o21, o22 = _out_combos([mm[t][a][b] for t in range(7)])
                        cc[a][b], cc[a][2 + b], cc[2 + a][b], cc[2 + a][2 + b] = o11, o12, o21, o22
                h = [[_silu(cc[q][b]) * cc[q][2 + b] for b in range(2)] for q in range(4)]
                return [[_pk(v) for v in _lhs_combos(h[a][0], h[a][1], h[2 + a][0], h[2 + a][1])] for a in range(2)]

            for q in range(4):
                x_copy(0, q).start()
            for c0 in range(NC0):
                for cp in w13_copies(c0, w13_0.at[c0], SEM_W0 + 4 * c0):
                    cp.start()
            for j in range(8, 24):
                qkv[j, 0:PAD, :] = jnp.zeros((PAD, 128), F32)
            for q in range(4):
                x_copy(0, q).wait()
            for i in range(1, NRP):
                for q in range(4):
                    x_copy(i, q).start()
            ln_store(0, ln_vals(0, False))
            for c0 in range(NC0):
                for cp in w13_copies(c0, w13_0.at[c0], SEM_W0 + 4 * c0):
                    cp.wait()
                for half in range(2):
                    rhs = first_rhs(w13_0.at[c0], half)
                    for t in range(7):
                        rg[c0, half, t] = rhs[t]
            for cp in w13_copies(NC0, w13_r.at[0], SEM_W):
                cp.start()
            for p in range(3):
                wqkv_copy(p).start()
            for n in range(8):
                w2_copy(n).start()
            for n in range(8):
                wo_copy(n).start()

            def first_body(i, carry):
                for ii in range(1, NRP):
                    @pl.when(i + 1 == ii)
                    def _():
                        for q in range(4):
                            x_copy(ii, q).wait()
                inext = jnp.where(i + 1 == NRP, 0, i + 1)
                rn = pl.multiple_of(inext * RQ, RQ)
                rh = pl.multiple_of(i * (RQ // 2), RQ // 2)
                rnh = pl.multiple_of(inext * (RQ // 2), RQ // 2)
                lhs_vals = [_unpk(jnp.concatenate([xl[t, pl.ds(rh, RQ // 2), :], xl[t, pl.ds(QS // 2 + rh, RQ // 2), :]], axis=0))
                            for t in range(7)]
                nxt = ln_vals(rn)
                for c0 in range(NC0):
                    ops = gate_up(lambda t: lhs_vals[t], c0)
                    for t in range(7):
                        pk = ops[t]
                        hl[c0, t, pl.ds(rh, RQ // 2), :] = pk[0:RQ // 2]
                        hl[c0, t, pl.ds(QS // 2 + rh, RQ // 2), :] = pk[RQ // 2:RQ]
                ln_store(rnh, nxt)
                return carry

            lax.fori_loop(0, NRP, first_body, 0)

            def qkv_tile(p, i):
                ln = lax.broadcasted_iota(jnp.int32, (D // 2, 128), 1)
                pos = (ln >> 2) & 7
                ys = []
                for j in range(8):
                    v = pltpu.bitcast(wqkv_r[p, :, j * 128:(j + 1) * 128], jnp.uint32)
                    ys.append(v if j == 0 else pltpu.roll(v, 4 * j, 1))
                hh_full = (ln >> 1) & 31
                base = ((hh_full & 3) * 8 + (hh_full >> 2))
                low = (ln >> 6) * 2 + (ln & 1)

                def column_tile(ii):
                    sel = (pos - ii) & 7
                    z = ys[0]
                    for j in range(1, 8):
                        z = jnp.where(sel == j, ys[j], z)
                    src = (((base + ii) & 31) << 2) + low
                    return jnp.take_along_axis(z, src, axis=1)

                left = column_tile(i)
                right = column_tile(i + 4)
                rhs = [_unpk(v) for v in _rhs_words(left[:QD], right[:QD], left[QD:], right[QD:])]
                c11, c12, c21, c22 = _out_combos(_products(lambda t: _unpk(xl[t]), rhs, ORDER))
                sc = jnp.where(p == 0, SCALE * LOG2E, 1.0).astype(F32)
                c11, c12, c21, c22 = c11 * sc, c12 * sc, c21 * sc, c22 * sc
                qkv[p * 8 + i, PAD:PAD + HS, :] = c11
                qkv[p * 8 + 4 + i, PAD:PAD + HS, :] = c12
                qkv[p * 8 + i, PAD + HS:PAD + S, :] = c21
                qkv[p * 8 + 4 + i, PAD + HS:PAD + S, :] = c22

            def main_body(jj, carry):
                j = jj + NC0
                slot = jj & 1
                for cp in w13_copies(j, w13_r.at[slot], SEM_W + 4 * slot):
                    cp.wait()
                for pp in range(3):
                    @pl.when(jj == 4 * pp)
                    def _():
                        wqkv_copy(pp).wait()

                @pl.when(jj + 1 < NMAIN)
                def _():
                    for cp in w13_copies(j + 1, w13_r.at[1 - slot], SEM_W + 4 * (1 - slot)):
                        cp.start()

                ops = gate_up2(w13_r.at[slot])
                for a in range(2):
                    for t in range(7):
                        hl[j, t, a * (QS // 2):(a + 1) * (QS // 2), :] = ops[a][t]
                qkv_tile(jj >> 2, jj & 3)
                return carry

            lax.fori_loop(0, NMAIN, main_body, 0)

        def phase_b(ol, b_v, out_v, wo_t):
            def attn_rows(r, masked, tok, never):
                ln = lax.broadcasted_iota(jnp.int32, (8, 128), 1)
                row = lax.broadcasted_iota(jnp.int32, (8, 128), 0) + r
                q = [qkv[j, pl.ds(r + PAD, 8), :] for j in range(8)]
                if tok is not None:
                    q = [jnp.where(never, tok, qq) for qq in q]
                logits = []
                for w in range(WIN):
                    p = None
                    for j in range(8):
                        t = q[j] * qkv[8 + j, pl.ds(r + (PAD - DIL * w), 8), :]
                        p = t if p is None else p + t
                    p = p + pltpu.roll(p, 64, 1)
                    p = p + jnp.take_along_axis(p, ln ^ 1, axis=1)
                    if w > 0 and masked:
                        p = jnp.where(row >= DIL * w, p, MASKED)
                    logits.append(p)
                mx = logits[0]
                for w in range(1, WIN):
                    mx = jnp.maximum(mx, logits[w])
                es = [jnp.exp2(l - mx) for l in logits]
                den = es[0]
                for w in range(1, WIN):
                    den = den + es[w]
                inv = 1.0 / den
                outs = []
                for j in range(8):
                    o = None
                    for w in range(WIN):
                        t = es[w] * qkv[16 + j, pl.ds(r + (PAD - DIL * w), 8), :]
                        o = t if o is None else o + t
                    outs.append(o * inv)
                return outs

            def attn_group(r, rh, masked, tok, never):
                res = []
                for hf in range(2):
                    pair = []
                    for e in range(2):
                        pair.append(attn_rows(hf * HS + r + 8 * e, masked and hf == 0, tok, never))
                    res.append(pair)
                tok = res[1][1][7]
                top, bot = res
                for j in range(4):
                    ops = _lhs_words(*[(v[0][c], v[1][c]) for v, c in ((top, j), (top, 4 + j), (bot, j), (bot, 4 + j))])
                    for t in range(7):
                        ol[t, pl.ds(rh, 8), j * 128:(j + 1) * 128] = ops[t]
                return tok

            def down_body(n, carry):
                wo_t[n, 0:HD, :] = _words(wo_r[n])
                wo_t[4 + n, 0:HD, :] = _words(wo_r[4 + n])
                a0h = pl.multiple_of(n * (AT_ROWS // 2), AT_ROWS // 2)
                a0 = pl.multiple_of(n * AT_ROWS, AT_ROWS)

                tok = None
                never = lax.broadcasted_iota(jnp.int32, (8, 128), 1) < (n - 1048576)
                for g in range(AT_ROWS // 16):
                    tok = attn_group(a0 + g * 16, a0h + g * 8, g == 0, tok, never)
                rhs = _rhs_combos(w2_r[n, 0:HF, :], w2_r[4 + n, 0:HF, :], w2_r[n, HF:F, :], w2_r[4 + n, HF:F, :])
                lhs = lambda t: jnp.concatenate([_unpk(hl[j, t]) for j in range(NCH)], axis=1)
                c11, c12, c21, c22 = _out_combos(_products(lhs, rhs, ORDER))
                b_v[n, 0:HS, :] = c11
                b_v[4 + n, 0:HS, :] = c12
                b_v[n, HS:S, :] = c21
                b_v[4 + n, HS:S, :] = c22
                return carry

            for n in range(8):
                w2_copy(n).wait()
                wo_copy(n).wait()
            lax.fori_loop(0, 4, down_body, 0)

            def out_copy(tile, half):
                c = pl.multiple_of(tile * 128, 128)
                return pltpu.make_async_copy(out_v.at[tile, pl.ds(half * HS, HS)],
                                             out_hbm.at[pl.ds(half * HS, HS), pl.ds(c, 128)], osem.at[tile * 2 + half])

            def fin_body(n, carry):
                def rows(tile, lo):
                    parts = [wo_t[tile, pl.ds(dd, 32, stride=16), :] for dd in range(lo, lo + 8)]
                    return jnp.concatenate(parts, axis=0)
                rhs = [_unpk(v) for v in _rhs_words(rows(n, 0), rows(4 + n, 0), rows(n, 8), rows(4 + n, 8))]
                s_q = _out_combos(_products(lambda t: _unpk(ol[t]), rhs, ORDER))
                quads = ((n, 0), (4 + n, 0), (n, 1), (4 + n, 1))
                for k in (1, 2, 3, 0):
                    tile, half = quads[k]
                    c = pl.multiple_of(tile * 128, 128)
                    rs = pl.ds(half * HS, HS)
                    g = _silu(b_v[tile, rs, :])
                    out_v[tile, rs, :] = (x_v[rs, pl.ds(c, 128)].astype(F32) + s_q[k] * g).astype(BF16)
                    out_copy(tile, half).start()
                return carry

            lax.fori_loop(0, 4, fin_body, 0)
            for tile in range(8):
                for half in range(2):
                    out_copy(tile, half).wait()

        pl.run_scoped(phase_a, *scoped_a)
        pl.run_scoped(phase_b, *scoped_b)

    scoped_a = [
        pltpu.VMEM((7, HS // 2, HD), jnp.uint32),
        pltpu.VMEM((49, S // 8, QD), jnp.uint32),
        pltpu.VMEM((NC0, 2, 7, HD // 2, 128), jnp.uint32),
        pltpu.VMEM((3, D, D), BF16),
        pltpu.VMEM((NC0, 4, D, 128), BF16),
        pltpu.VMEM((2, 4, D, 128), BF16),
    ]
    scoped_b = [
        pltpu.VMEM((7, HS // 2, HD), jnp.uint32),
        pltpu.VMEM((8, S, 128), F32),
        pltpu.VMEM((8, S, 128), BF16),
        pltpu.VMEM((8, D // 2 + 16, 128), jnp.uint32),
    ]
    scratch = [
        pltpu.VMEM((S, D), BF16),
        pltpu.VMEM((8, F, 128), BF16),
        pltpu.VMEM((8, D, 128), BF16),
        pltpu.VMEM((NCH, 7, HS // 2, 128), jnp.uint32),
        pltpu.VMEM((24, S + PAD, 128), F32),
        pltpu.SemaphoreType.DMA((4 * NRP + 3 + 4 * NC0 + 24,)),
        pltpu.SemaphoreType.DMA((16,)),
    ]
    return kernel, scratch


@jax.jit
def pallas_recurrent_scan__sliding_local_dilated__glu_gated_swiglu__prompt_kernel(
    A_x: jax.Array,
    A_wqkv: jax.Array,
    A_wo: jax.Array,
    B_x: jax.Array,
    B_w1: jax.Array,
    B_w3: jax.Array,
    B_w2: jax.Array,
):
    del B_x
    kernel, scratch = _make_kernel()
    any_spec = pl.BlockSpec(memory_space=pl.ANY)
    out = pl.pallas_call(
        kernel,
        out_shape=jax.ShapeDtypeStruct((S, D), BF16),
        in_specs=[any_spec] * 6,
        out_specs=any_spec,
        scratch_shapes=scratch,
        compiler_params=pltpu.CompilerParams(
            vmem_limit_bytes=120 * 2**20,
            flags={"XLA_TPU_EVENLY_DISTRIBUTE_CRITICAL_NODES": True},
        ),
    )(A_x.reshape(S, D), A_wqkv, A_wo, B_w1, B_w3, B_w2)
    return out.reshape(1, S, D)
```
